```python
import os as _os
_os.environ.setdefault("JAX_PLATFORMS", "cpu")
import jax
import jax.numpy as jnp

def _softmax(x, axis=-1):
    return jax.nn.softmax(x, axis=axis)
def _gelu(x):
    return jax.nn.gelu(x, approximate=True)
def _silu(x):
    return jax.nn.silu(x)
def _sigmoid(x):
    return jax.nn.sigmoid(x)
def _layernorm(x, axis=-1, eps=1e-5):
    m = jnp.mean(x, axis=axis, keepdims=True)
    v = jnp.var(x, axis=axis, keepdims=True)
    return (x - m) / jnp.sqrt(v + eps)
def _scatter_add(tgt, idx, src, axis=0):
    return tgt.at[idx].add(src)
def _segment_sum(src, seg, n):
    return jax.ops.segment_sum(src, seg, n)
class _Rng:
    def __init__(self, key):
        self._k = key
    def _next(self):
        self._k, sub = jax.random.split(self._k)
        return sub
    def normal(self, shape):
        return jax.random.normal(self._next(), shape, dtype=jnp.bfloat16)
    def randint(self, lo, hi, shape):
        return jax.random.randint(self._next(), shape, lo, hi, dtype=jnp.int32)
    def uniform(self, shape, lo=0.0, hi=1.0):
        return jax.random.uniform(self._next(), shape, jnp.bfloat16, lo, hi)
    def permutation(self, n):
        return jax.random.permutation(self._next(), n)


kernel_name = 'sequential_preLN__softmax_full_mha__glu_gated_swiglu__prompt'

def setup_inputs():
    _rng = _Rng(jax.random.key(int.from_bytes(__import__("os").urandom(4), "little")))
    _w = (lambda a: (lambda t: t.astype(jnp.bfloat16) if jnp.issubdtype(t.dtype, jnp.floating) else t)(jnp.asarray(a)))
    def _A_setup():
        B, S, D = 1, 2048, 640
        return {
            "x": _w((lambda *s: _rng.normal(s) * 0.05)(B, S, D)),
            "wqkv": _w((lambda *s: _rng.normal(s) * 0.05)(D, 3 * D)),
            "wo": _w((lambda *s: _rng.normal(s) * 0.05)(D, D)),
        }
    _A_in = _A_setup()

    def _B_setup():
        B, S, D, F = 1, 2048, 640, 1728
        return {
            "x": _w((lambda *s: _rng.normal(s) * 0.05)(B, S, D)),
            "w1": _w((lambda *s: _rng.normal(s) * 0.05)(D, F) * (2.0 / D) ** 0.5),
            "w3": _w((lambda *s: _rng.normal(s) * 0.05)(D, F) * (2.0 / D) ** 0.5),
            "w2": _w((lambda *s: _rng.normal(s) * 0.05)(F, D) * (2.0 / F) ** 0.5),
        }
    _B_in = _B_setup()

    return {
        "A_x": _A_in["x"],
        "A_wqkv": _A_in["wqkv"],
        "A_wo": _A_in["wo"],
        "B_x": _B_in["x"],
        "B_w1": _B_in["w1"],
        "B_w3": _B_in["w3"],
        "B_w2": _B_in["w2"],
    }

def reference(A_x, A_wqkv, A_wo, B_x, B_w1, B_w3, B_w2):
    def _A_ref(x, wqkv, wo):
        B, S, D = x.shape
        H = 32; Dh = D // H
        qkv = (lambda x, *d: x.transpose(*d))((x @ wqkv).reshape(B, S, 3, H, Dh), 2, 0, 3, 1, 4)
        q, k, v = qkv[0], qkv[1], qkv[2]
        scale = Dh ** -0.5
        scores = jnp.einsum("bhqd,bhkd->bhqk", q, k) * scale
        p = _softmax(scores, axis=-1)
        o = jnp.einsum("bhqk,bhkd->bhqd", p, v)
        return (lambda x, *d: x.transpose(*d))(o, 0, 2, 1, 3).reshape(B, S, D) @ wo

    def _B_ref(x, w1, w3, w2):
        gate = jnp.einsum("bsd,df->bsf", x, w1)
        up = jnp.einsum("bsd,df->bsf", x, w3)
        h = _silu(gate) * up
        out = jnp.einsum("bsf,fd->bsd", h, w2)
        return out

    x = A_x
    h = x + _A_ref(_layernorm(x, axis=-1), A_wqkv, A_wo)
    h2 = h + _B_ref(_layernorm(h, axis=-1), B_w1, B_w3, B_w2)
    return h2
```

```python
import functools
import jax
import jax.numpy as jnp
import numpy as np
from jax import lax
import jax.experimental.pallas as pl
import jax.experimental.pallas.tpu as pltpu

S, D, H, DH, F = 2048, 640, 32, 20, 1728
NSL = 6
FP = 1792
EPS = 1e-5
LOG2E = 1.4426950408889634
QSCALE = (DH ** -0.5) * LOG2E
L_LO, L_HI = 2.0 ** -60, 2.0 ** 60
BF = jnp.bfloat16
F32 = jnp.float32

TB = 512
TQ = 1024
BJ = 1024
TM = 512
SCOPES = False

import contextlib
def scope(name):
    return jax.named_scope(name) if SCOPES else contextlib.nullcontext()

def _ln(x):
    mu = jnp.mean(x, axis=-1, keepdims=True)
    xc = x - mu
    var = jnp.mean(xc * xc, axis=-1, keepdims=True)
    return xc * lax.rsqrt(var + EPS)

def _dot(a, b):
    return jnp.dot(a, b, preferred_element_type=F32)

def _dot_nt(a, b):
    return lax.dot_general(a, b, (((1,), (1,)), ((), ())), preferred_element_type=F32)

def _kernel(x_hbm, wqkv_hbm, wo_hbm, w1t_hbm, w3t_hbm, w2_hbm, out_hbm,
            x_s, wqkv_s, wo_s, w13_s, w2_s, wk_s, wqvT_s, k_s, q_s, nq_s, vt_s, ot_s, ob_s, sems):
    NXB = S // TB
    x_cp = [pltpu.make_async_copy(x_hbm.at[pl.ds(b * TB, TB)], x_s.at[pl.ds(b * TB, TB)], sems.at[b]) for b in range(NXB)]
    o = NXB
    wqkv_cp = pltpu.make_async_copy(wqkv_hbm, wqkv_s, sems.at[o])
    wo_cp = pltpu.make_async_copy(wo_hbm, wo_s, sems.at[o + 1])
    FM = 1664
    w13_cps = [
        pltpu.make_async_copy(w1t_hbm.at[pl.ds(0, FM)], w13_s.at[pl.ds(0, FM)], sems.at[o + 2]),
        pltpu.make_async_copy(w3t_hbm.at[pl.ds(0, FM)], w13_s.at[pl.ds(FM, FM)], sems.at[o + 3]),
        pltpu.make_async_copy(w1t_hbm.at[pl.ds(FM, F - FM)], w13_s.at[pl.ds(2 * FM, F - FM)], sems.at[o + 4]),
        pltpu.make_async_copy(w3t_hbm.at[pl.ds(FM, F - FM)], w13_s.at[pl.ds(2 * FM + F - FM, F - FM)], sems.at[o + 5]),
    ]
    w2_cp = pltpu.make_async_copy(w2_hbm, w2_s.at[pl.ds(0, F)], sems.at[o + 6])
    NOB = S // TM
    out_cp = [pltpu.make_async_copy(ob_s.at[b], out_hbm.at[pl.ds(b * TM, TM)], sems.at[o + 7 + b]) for b in range(NOB)]

    wqkv_cp.start()
    for cp in x_cp:
        cp.start()
    wo_cp.start()
    for cp in w13_cps:
        cp.start()
    w2_cp.start()
    w2_s[F:FP, :] = jnp.zeros((FP - F, D), BF)

    with scope('P1a'):
        wqkv_cp.wait()
        for c in range(NSL):
            wk_s[:, c * 128:(c + 1) * 128] = wqkv_s[:, D + 120 * c: D + 120 * c + 128]
        wqvT_s[0:D, :] = wqkv_s[:, 0:D].T
        wqvT_s[D:2 * D, :] = wqkv_s[:, 2 * D:3 * D].T

    lane = lax.broadcasted_iota(jnp.int32, (TB, 128), 1)
    l8 = lax.broadcasted_iota(jnp.int32, (8, 128), 1)
    segk = jnp.where((l8 // DH == lax.broadcasted_iota(jnp.int32, (8, 128), 0)) & (l8 < 120), 1.0, 0.0).astype(BF)
    r = lax.broadcasted_iota(jnp.int32, (48, D), 0)
    f = lax.broadcasted_iota(jnp.int32, (48, D), 1)
    segq = jnp.where(((r % 8) < 6) & (f // DH == 6 * (r // 8) + (r % 8)), 1.0, 0.0).astype(BF)
    ones8 = jnp.ones((8, TB), F32)

    kmx = [jnp.zeros((8, 128), F32) for _ in range(NSL)]
    with scope('P1b'):
      for b in range(NXB):
        t0 = b * TB
        x_cp[b].wait()
        xn = _ln(x_s[t0:t0 + TB, :].astype(F32)).astype(BF)
        kk = _dot(xn, wk_s[...])
        for c in range(NSL):
            kc = jnp.where(lane >= 120, 1.0, kk[:, c * 128:(c + 1) * 128]).astype(BF)
            k_s[c, t0:t0 + TB, :] = kc
            kf = kc.astype(F32)
            nsq = _dot_nt(segk, (kf * kf).astype(BF))
            m = nsq[:, 0:128]
            for t in range(1, TB // 128):
                m = jnp.maximum(m, nsq[:, t * 128:(t + 1) * 128])
            kmx[c] = jnp.maximum(kmx[c], m)
        qv = _dot_nt(wqvT_s[...], xn)
        qf = (qv[0:D, :] * QSCALE).astype(BF).astype(F32)
        nq_s[:, t0:t0 + TB] = _dot(segq, (qf * qf).astype(BF))
        for c in range(NSL):
            lo = 120 * c
            hi = min(lo + 120, D)
            q_s[c, 0:hi - lo, t0:t0 + TB] = qf[lo:hi, :]
            if hi - lo < 120:
                q_s[c, hi - lo:120, t0:t0 + TB] = jnp.zeros((120 - (hi - lo), TB), F32)
        vT = qv[D:2 * D, :]
        for h in range(H):
            a = 8 * ((DH * h) // 8)
            blk = jnp.concatenate([vT[a:a + 24, :], ones8], axis=0).astype(BF)
            for jt in range(TB // 128):
                vt_s[h * 16 + b * (TB // 128) + jt] = blk[:, jt * 128:(jt + 1) * 128]
    with scope('P1c'):
        for c in range(NSL):
            kmax = jnp.sqrt(jnp.max(kmx[c], axis=1, keepdims=True))
            q_s[c, 120:128, :] = -(jnp.sqrt(nq_s[8 * c:8 * c + 8, :]) * kmax) * (1.0 + 2.0 ** -6)

    qrow = lax.broadcasted_iota(jnp.int32, (128, 128), 0)

    def qtile(c, p, q0, tq, with_b):
        m = (qrow >= DH * p) & (qrow < DH * p + DH)
        if with_b:
            m = m | (qrow == 120 + p)
        parts = []
        for t in range(tq // 128):
            if isinstance(q0, int):
                qi = q_s[c, :, q0 + t * 128:q0 + (t + 1) * 128]
            else:
                qi = q_s[c, :, pl.ds(q0 + t * 128, 128)]
            parts.append(jnp.where(m, qi, 0.0).astype(BF))
        return jnp.concatenate(parts, axis=1)

    def store_pair(u, q0, tq, acc_e, acc_o):
        sub = lax.broadcasted_iota(jnp.int32, (8, tq), 0)
        ie = 1.0 / acc_e[24:32, :]
        io = 1.0 / acc_o[24:32, :]
        mid = jnp.where(sub < 4, acc_e[16:24, :] * ie, acc_o[0:8, :] * io)
        blk = jnp.concatenate([acc_e[0:8, :] * ie, acc_e[8:16, :] * ie, mid,
                               acc_o[8:16, :] * io, acc_o[16:24, :] * io], axis=0)
        if isinstance(q0, int):
            ot_s[pl.ds(pl.multiple_of(u * 40, 8), 40), q0:q0 + tq] = blk
        else:
            ot_s[pl.ds(pl.multiple_of(u * 40, 8), 40), pl.ds(q0, tq)] = blk

    def pair_body(u, bad):
        c = u // 3
        up = u % 3
        for qb in range(S // TQ):
            accs = []
            for e in range(2):
                p = 2 * up + e
                h = 2 * u + e
                qt = qtile(c, p, qb * TQ, TQ, True)
                acc = jnp.zeros((32, TQ), F32)
                for jb in range(S // BJ):
                    s = _dot(k_s[c, jb * BJ:(jb + 1) * BJ, :], qt)
                    pT = jnp.exp2(s).astype(BF)
                    v = jnp.concatenate([vt_s[h * 16 + jb * (BJ // 128) + t] for t in range(BJ // 128)], axis=1)
                    acc = acc + _dot(v, pT)
                accs.append(acc)
                l = acc[24:32, :]
                bad = jnp.maximum(bad, jnp.where((l >= L_LO) & (l <= L_HI), 0.0, 1.0))
            store_pair(u, qb * TQ, TQ, accs[0], accs[1])
        return bad

    with scope('P2'):
        bad = lax.fori_loop(0, H // 2, pair_body, jnp.zeros((8, TQ), F32))
    flag = jnp.max(bad)

    @pl.when(flag > 0.0)
    def _slow():
        tq, bj = 256, 512
        def body(it, carry):
            u = it // (S // tq)
            q0 = pl.multiple_of((it % (S // tq)) * tq, tq)
            c = u // 3
            up = u % 3
            accs = []
            for e in range(2):
                p = 2 * up + e
                h = 2 * u + e
                qt = qtile(c, p, q0, tq, False)
                def mx(jb, m):
                    j0 = pl.multiple_of(jb * bj, bj)
                    s = _dot(k_s[c, pl.ds(j0, bj), :], qt)
                    return jnp.maximum(m, jnp.max(s, axis=0, keepdims=True))
                m = lax.fori_loop(0, S // bj, mx, jnp.full((1, tq), -jnp.inf, F32))
                def pv(jb, acc):
                    j0 = pl.multiple_of(jb * bj, bj)
                    s = _dot(k_s[c, pl.ds(j0, bj), :], qt)
                    pT = jnp.exp2(s - m).astype(BF)
                    v = jnp.concatenate([vt_s[h * 16 + jb * (bj // 128) + t] for t in range(bj // 128)], axis=1)
                    return acc + _dot(v, pT)
                accs.append(lax.fori_loop(0, S // bj, pv, jnp.zeros((32, tq), F32)))
            store_pair(u, q0, tq, accs[0], accs[1])
            return carry
        lax.fori_loop(0, (H // 2) * (S // tq), body, 0)

    wo_cp.wait()
    for cp in w13_cps:
        cp.wait()
    w2_cp.wait()
    lane_m = lax.broadcasted_iota(jnp.int32, (TM, 128), 1)

    def ffn_block(rb):
        r0 = rb * TM
        oT = ot_s[:, r0:r0 + TM].astype(BF)
        a = lax.dot_general(oT, wo_s[...], (((0,), (0,)), ((), ())), preferred_element_type=F32)
        hres = x_s[r0:r0 + TM, :].astype(F32) + a
        hn = _ln(hres).astype(BF)
        gu = _dot_nt(hn, w13_s[...])
        g = gu[:, 0:FM]
        up_ = gu[:, FM:2 * FM]
        act_main = (g * jax.nn.sigmoid(g) * up_).astype(BF)
        t = gu[:, 2 * FM:2 * FM + 128]
        act_last = jnp.where(lane_m < 64, t * jax.nn.sigmoid(t) * pltpu.roll(t, 64, 1), 0.0).astype(BF)
        act = jnp.concatenate([act_main, act_last], axis=1)
        y = hres + _dot(act, w2_s[...])
        ob_s[rb] = y.astype(BF)
        out_cp[rb].start()

    with scope('P3'):
        for rb in range(NOB):
            ffn_block(rb)
    for cp in out_cp:
        cp.wait()


@jax.jit
def pallas_sequential_preLN__softmax_full_mha__glu_gated_swiglu__prompt_kernel(A_x, A_wqkv, A_wo, B_x, B_w1, B_w3, B_w2):
    del B_x
    x = A_x.reshape(S, D)
    nsem = S // TB + 7 + S // TM
    hbm = pl.BlockSpec(memory_space=pltpu.HBM)
    out = pl.pallas_call(
        _kernel,
        out_shape=jax.ShapeDtypeStruct((S, D), A_x.dtype),
        in_specs=[hbm] * 6,
        out_specs=hbm,
        scratch_shapes=[
            pltpu.VMEM((S, D), BF),
            pltpu.VMEM((D, 3 * D), BF),
            pltpu.VMEM((D, D), BF),
            pltpu.VMEM((2 * F, D), BF),
            pltpu.VMEM((FP, D), BF),
            pltpu.VMEM((D, NSL * 128), BF),
            pltpu.VMEM((2 * D, D), BF),
            pltpu.VMEM((NSL, S, 128), BF),
            pltpu.VMEM((NSL, 128, S), F32),
            pltpu.VMEM((48, S), F32),
            pltpu.VMEM((H * 16, 32, 128), BF),
            pltpu.VMEM((D, S), F32),
            pltpu.VMEM((S // TM, TM, D), BF),
            pltpu.SemaphoreType.DMA((nsem,)),
        ],
        compiler_params=pltpu.CompilerParams(vmem_limit_bytes=110 * 1024 * 1024),
        name="fused_block",
    )(x, A_wqkv, A_wo, B_w1.T, B_w3.T, B_w2)
    return out.reshape(A_x.shape)
```

```python
import functools
import jax
import jax.numpy as jnp
import numpy as np
from jax import lax
import jax.experimental.pallas as pl
import jax.experimental.pallas.tpu as pltpu

S, D, H, DH, F = 2048, 640, 32, 20, 1728
NSL = 6
FP = 1792
EPS = 1e-5
LOG2E = 1.4426950408889634
QSCALE = (DH ** -0.5) * LOG2E
L_LO, L_HI = 2.0 ** -90, 2.0 ** 60
BF = jnp.bfloat16
F32 = jnp.float32

TB = 512
TQ = 512
BJ = 128
LAG = 4
HU = 4
TM = 512
KSHIFT = 1
WSTART = 0
PH = '123'
P1V = 4
PST = 1
SCOPES = False

import contextlib
def scope(name):
    return jax.named_scope(name) if SCOPES else contextlib.nullcontext()

def _ln(x):
    mu = jnp.mean(x, axis=-1, keepdims=True)
    xc = x - mu
    var = jnp.mean(xc * xc, axis=-1, keepdims=True)
    return xc * lax.rsqrt(var + EPS)

def _dot(a, b):
    return lax.dot_general(a, b, (((1,), (0,)), ((), ())), preferred_element_type=F32)

def _dot_nt(a, b):
    return lax.dot_general(a, b, (((1,), (1,)), ((), ())), preferred_element_type=F32)

def _kernel(x_hbm, wqkv_hbm, wo_hbm, w1t_hbm, w3t_hbm, w2_hbm, out_hbm,
            x_s, xn_s, wqkv_s, wo_s, w13_s, w2_s, wk_s, wqvT_s, k_s, q_s, nq_s, vt_s, ot_s, ob_s, p_s, sems):
    NXB = S // TB
    XP = [int(t) for t in '0,512,1024,2048'.split(',')] if P1V == 4 else [b * TB for b in range(NXB + 1)]
    x_cp = [pltpu.make_async_copy(x_hbm.at[pl.ds(XP[b], XP[b + 1] - XP[b])], x_s.at[pl.ds(XP[b], XP[b + 1] - XP[b])], sems.at[b]) for b in range(len(XP) - 1)]
    o = 8
    def wcols(c0, n, si):
        return pltpu.make_async_copy(wqkv_hbm.at[:, pl.ds(c0, n)], wqkv_s.at[:, pl.ds(c0, n)], sems.at[si])
    wk_cp = wcols(D, D, o)
    wq_cp = wcols(0, D, o + 1)
    wv_cp = wcols(2 * D, D, o + 2)
    o += 3
    wo_cp = pltpu.make_async_copy(wo_hbm, wo_s, sems.at[o])
    FM = 1664
    w13_cps = [
        pltpu.make_async_copy(w1t_hbm.at[pl.ds(0, FM)], w13_s.at[pl.ds(0, FM)], sems.at[o + 1]),
        pltpu.make_async_copy(w3t_hbm.at[pl.ds(0, FM)], w13_s.at[pl.ds(FM, FM)], sems.at[o + 2]),
        pltpu.make_async_copy(w1t_hbm.at[pl.ds(FM, F - FM)], w13_s.at[pl.ds(2 * FM, F - FM)], sems.at[o + 3]),
        pltpu.make_async_copy(w3t_hbm.at[pl.ds(FM, F - FM)], w13_s.at[pl.ds(2 * FM + F - FM, F - FM)], sems.at[o + 4]),
    ]
    w2_cp = pltpu.make_async_copy(w2_hbm, w2_s.at[pl.ds(0, F)], sems.at[o + 5])
    NOB = S // TM
    out_cp = [pltpu.make_async_copy(ob_s.at[b], out_hbm.at[pl.ds(b * TM, TM)], sems.at[o + 6 + b]) for b in range(NOB)]

    lane = lax.broadcasted_iota(jnp.int32, (TB, 128), 1)
    rk = lax.broadcasted_iota(jnp.int32, (48, NSL * 128), 0)
    lk = lax.broadcasted_iota(jnp.int32, (48, NSL * 128), 1)
    segk = jnp.where((lk // 128 == rk // 8) & ((lk % 128) // DH == rk % 8) & (lk % 128 < 120), 1.0, 0.0).astype(BF)
    r = lax.broadcasted_iota(jnp.int32, (48, D), 0)
    f = lax.broadcasted_iota(jnp.int32, (48, D), 1)
    segq = jnp.where(((r % 8) < 6) & (f // DH == 6 * (r // 8) + (r % 8)), 1.0, 0.0).astype(BF)
    kmx = [jnp.zeros((48, 128), F32)]

    def ln1(b):
        t0 = b * TB
        xn_s[t0:t0 + TB, :] = _ln(x_s[t0:t0 + TB, :].astype(F32)).astype(BF)

    def kproj(b):
        t0 = b * TB
        xn = xn_s[t0:t0 + TB, :]
        if KSHIFT:
            kk = _dot(xn, wqkv_s[:, D:2 * D]).astype(BF)
            kk = jnp.concatenate([kk, jnp.zeros((TB, 128), BF)], axis=1)
        else:
            kk = _dot(xn, wk_s[...])
        for c in range(NSL):
            if KSHIFT:
                kc = kk[:, 120 * c:120 * c + 128]
                kc = jnp.where(lane >= 120, jnp.ones_like(kc), kc)
            else:
                kc = jnp.where(lane >= 120, 1.0, kk[:, c * 128:(c + 1) * 128]).astype(BF)
            k_s[c, t0:t0 + TB, :] = kc

    def knorm(b):
        t0 = b * TB
        kf = jnp.concatenate([k_s[c, t0:t0 + TB, :] for c in range(NSL)], axis=1).astype(F32)
        nsq = _dot_nt(segk, (kf * kf).astype(BF))
        m = nsq[:, 0:128]
        for t in range(1, TB // 128):
            m = jnp.maximum(m, nsq[:, t * 128:(t + 1) * 128])
        kmx[0] = jnp.maximum(kmx[0], m)

    def qvproj(b):
        t0 = b * TB
        xn = xn_s[t0:t0 + TB, :]
        qv = _dot_nt(wqvT_s[...], xn)
        qf = (qv[0:D, :] * QSCALE).astype(BF).astype(F32)
        nq_s[:, t0:t0 + TB] = _dot(segq, (qf * qf).astype(BF))
        for c in range(NSL):
            lo = 120 * c
            hi = min(lo + 120, D)
            q_s[c, 0:hi - lo, t0:t0 + TB] = qf[lo:hi, :]
            if hi - lo < 120:
                q_s[c, hi - lo:120, t0:t0 + TB] = jnp.zeros((120 - (hi - lo), TB), F32)
        vT = qv[D:2 * D, :].astype(BF).astype(F32)
        sub = lax.broadcasted_iota(jnp.int32, (8, TB), 0)
        for h in range(H):
            a = 8 * ((DH * h) // 8)
            if h % 2 == 0:
                blk = jnp.concatenate([vT[a:a + 16, :], jnp.where(sub < 4, vT[a + 16:a + 24, :], 1.0)], axis=0)
            else:
                blk = jnp.concatenate([jnp.where(sub < 4, 1.0, vT[a:a + 8, :]), vT[a + 8:a + 24, :]], axis=0)
            for jt in range(TB // 128):
                vt_s[h * 16 + b * (TB // 128) + jt] = blk[:, jt * 128:(jt + 1) * 128]

    WPRI = 1
    def start_w():
        wo_cp.start(priority=WPRI)
        for cp in w13_cps:
            cp.start(priority=WPRI)
        w2_cp.start(priority=WPRI)

    if P1V == 4:
        XORD = 1
        if XORD == 0:
            wk_cp.start()
            for cp in x_cp:
                cp.start()
        else:
            x_cp[0].start()
            wk_cp.start()
            for cp in x_cp[1:]:
                cp.start()
    else:
        x_cp[0].start()
        wk_cp.start()
        for cp in x_cp[1:]:
            cp.start()
    wq_cp.start()
    wv_cp.start()
    start_w()
    def transp():
        wqvT_s[0:D, :] = wqkv_s[:, 0:D].T
        wqvT_s[D:2 * D, :] = wqkv_s[:, 2 * D:3 * D].T

    def kmm(b):
        t0 = b * TB
        return _dot(xn_s[t0:t0 + TB, :], wqkv_s[:, D:2 * D])

    def kpost(b, kk):
        t0 = b * TB
        kk = kk.astype(BF)
        kk = jnp.concatenate([kk, jnp.zeros((TB, 128), BF)], axis=1)
        for c in range(NSL):
            kc = kk[:, 120 * c:120 * c + 128]
            kc = jnp.where(lane >= 120, jnp.ones_like(kc), kc)
            k_s[c, t0:t0 + TB, :] = kc

    w2_s[F:FP, :] = jnp.zeros((FP - F, D), BF)
    if P1V == 0:
      with scope('P1a'):
        x_cp[0].wait()
        ln1(0)
        wk_cp.wait()
        x_cp[1].wait()
        ln1(1)
        kproj(0)
        x_cp[2].wait()
        x_cp[3].wait()
        ln1(2)
        ln1(3)
        kproj(1)
      with scope('P1b'):
        wq_cp.wait()
        wv_cp.wait()
        transp()
        kproj(2)
        kproj(3)
        for b in range(NXB):
            qvproj(b)
            knorm(b)
    elif P1V == 1:
      with scope('P1a'):
        x_cp[0].wait()
        ln1(0)
        wk_cp.wait()
        x_cp[1].wait()
        k0 = kmm(0)
        ln1(1)
        kpost(0, k0)
        x_cp[2].wait()
        x_cp[3].wait()
        k1 = kmm(1)
        ln1(2)
        ln1(3)
        kpost(1, k1)
      with scope('P1b'):
        wq_cp.wait()
        wv_cp.wait()
        k2 = kmm(2)
        transp()
        k3 = kmm(3)
        kpost(2, k2)
        qvproj(0)
        kpost(3, k3)
        knorm(0)
        for b in range(1, NXB):
            qvproj(b)
            knorm(b)
    elif P1V == 2:
      with scope('P1a'):
        x_cp[0].wait()
        ln1(0)
        x_cp[1].wait()
        ln1(1)
        wk_cp.wait()
        k0 = kmm(0)
        kpost(0, k0)
        k1 = kmm(1)
        x_cp[2].wait()
        x_cp[3].wait()
        ln1(2)
        kpost(1, k1)
        k2 = kmm(2)
        ln1(3)
      with scope('P1b'):
        wq_cp.wait()
        wv_cp.wait()
        k3 = kmm(3)
        kpost(2, k2)
        transp()
        kpost(3, k3)
        for b in range(NXB):
            qvproj(b)
            knorm(b)
    elif P1V == 3:
      RC = 128
      LC = 128
      NC = S // RC
      def lnc(i):
        for t0 in range(i * RC, (i + 1) * RC, LC):
            xn_s[t0:t0 + LC, :] = _ln(x_s[t0:t0 + LC, :].astype(F32)).astype(BF)
      lanec = lax.broadcasted_iota(jnp.int32, (RC, 128), 1)
      def kc_(i):
        t0 = i * RC
        kk = _dot(xn_s[t0:t0 + RC, :], wqkv_s[:, D:2 * D]).astype(BF)
        kk = jnp.concatenate([kk, jnp.zeros((RC, 128), BF)], axis=1)
        for c in range(NSL):
            kc = kk[:, 120 * c:120 * c + 128]
            k_s[c, t0:t0 + RC, :] = jnp.where(lanec >= 120, jnp.ones_like(kc), kc)
      def tr(j):
        src_c = j * 128 if j < 5 else 2 * D + (j - 5) * 128
        wqvT_s[j * 128:(j + 1) * 128, :] = wqkv_s[:, src_c:src_c + 128].T
      PB = TB // RC
      with scope('P1a'):
        x_cp[0].wait()
        for i in range(PB):
            lnc(i)
        wk_cp.wait()
        x_cp[1].wait()
        for i in range(PB):
            kc_(i)
            lnc(PB + i)
        x_cp[2].wait()
        x_cp[3].wait()
        for i in range(PB):
            kc_(PB + i)
            lnc(2 * PB + i)
        for i in range(PB):
            kc_(2 * PB + i)
            lnc(3 * PB + i)
      with scope('P1b'):
        wq_cp.wait()
        wv_cp.wait()
        trs = list(range(10))
        per = (10 + PB - 1) // PB
        for i in range(PB):
            kc_(3 * PB + i)
            for j in trs[i * per:(i + 1) * per]:
                tr(j)
        for b in range(NXB):
            qvproj(b)
            knorm(b)
    elif P1V == 4:
      RC = 128
      LC = 64
      AH = 2
      NC = S // RC
      def lnc(i):
        for t0 in range(i * RC, (i + 1) * RC, LC):
            xn_s[t0:t0 + LC, :] = _ln(x_s[t0:t0 + LC, :].astype(F32)).astype(BF)
      lanec = lax.broadcasted_iota(jnp.int32, (RC, 128), 1)
      def kc_(i):
        t0 = i * RC
        kk = _dot(xn_s[t0:t0 + RC, :], wqkv_s[:, D:2 * D]).astype(BF)
        kk = jnp.concatenate([kk, jnp.zeros((RC, 128), BF)], axis=1)
        for c in range(NSL):
            kc = kk[:, 120 * c:120 * c + 128]
            k_s[c, t0:t0 + RC, :] = jnp.where(lanec >= 120, jnp.ones_like(kc), kc)
      def tr(j):
        src_c = j * 128 if j < 5 else 2 * D + (j - 5) * 128
        wqvT_s[j * 128:(j + 1) * 128, :] = wqkv_s[:, src_c:src_c + 128].T
      piece = [0]
      def need(i):
        while XP[piece[0]] < (i + 1) * RC:
            x_cp[piece[0]].wait()
            piece[0] += 1
      TRS = 12
      with scope('P1a'):
        if XORD == 0:
            wk_cp.wait()
        for i in range(AH):
            need(i)
            lnc(i)
        if XORD != 0:
            wk_cp.wait()
        trs = list(range(10))
        for i in range(NC):
            if i + AH < NC:
                need(i + AH)
            if i == TRS:
                wq_cp.wait()
                wv_cp.wait()
            kc_(i)
            if i + AH < NC:
                lnc(i + AH)
            if i >= TRS:
                left = NC - i
                n = (len(trs) + left - 1) // left
                for j in trs[:n]:
                    tr(j)
                trs = trs[n:]
      with scope('P1b'):
        for b in range(NXB):
            qvproj(b)
            knorm(b)
    with scope('P1c'):
        for c in range(NSL):
            kmax = jnp.sqrt(jnp.max(kmx[0][8 * c:8 * c + 8, :], axis=1, keepdims=True))
            q_s[c, 120:128, :] = -(jnp.sqrt(nq_s[8 * c:8 * c + 8, :]) * kmax) * (1.0 + 2.0 ** -6)

    if WSTART == 1:
        start_w()
    qrow = lax.broadcasted_iota(jnp.int32, (128, 128), 0)

    def qtile(c, p, q0, tq, with_b):
        m = (qrow >= DH * p) & (qrow < DH * p + DH)
        if with_b:
            m = m | (qrow == 120 + p)
        parts = []
        for t in range(tq // 128):
            if isinstance(q0, int):
                qi = q_s[c, :, q0 + t * 128:q0 + (t + 1) * 128]
            else:
                qi = q_s[c, :, pl.ds(q0 + t * 128, 128)]
            parts.append(jnp.where(m, qi, 0.0).astype(BF))
        return jnp.concatenate(parts, axis=1)

    def store_pair(u, q0, tq, acc_e, acc_o):
        sub = lax.broadcasted_iota(jnp.int32, (8, tq), 0)
        le = jnp.broadcast_to(acc_e[20:21, :], (8, tq))
        lo = jnp.broadcast_to(acc_o[0:1, :], (8, tq))
        ie = 1.0 / le
        io = 1.0 / lo
        mid = jnp.where(sub < 4, acc_e[16:24, :] * ie, acc_o[0:8, :] * io)
        blk = jnp.concatenate([acc_e[0:8, :] * ie, acc_e[8:16, :] * ie, mid,
                               acc_o[8:16, :] * io, acc_o[16:24, :] * io], axis=0)
        if isinstance(q0, int):
            ot_s[pl.ds(pl.multiple_of(u * 40, 8), 40), q0:q0 + tq] = blk
        else:
            ot_s[pl.ds(pl.multiple_of(u * 40, 8), 40), pl.ds(q0, tq)] = blk
        mn = jnp.minimum(le, lo)
        mx = jnp.maximum(le, lo)
        okv = jnp.where((mn >= L_LO) & (mx <= L_HI) & (le <= L_HI) & (lo <= L_HI), 0.0, 1.0)
        r = okv[:, 0:128]
        for t in range(1, tq // 128):
            r = jnp.maximum(r, okv[:, t * 128:(t + 1) * 128])
        return r

    def attn_body(it, bad):
        items = [(us, qb, e, jb) for us in range(HU // 2) for qb in range(S // TQ)
                 for e in range(2) for jb in range(S // BJ)]
        qts, P, acc = {}, {}, {}
        cnt = [0]
        st = [bad]

        def do_qk(us, qb, e, jb):
            u = it * (HU // 2) + us
            c = u // 3
            p = 2 * (u % 3) + e
            if (us, qb, e) not in qts:
                qts[(us, qb, e)] = qtile(c, p, qb * TQ, TQ, True)
            s = _dot(k_s[c, jb * BJ:(jb + 1) * BJ, :], qts[(us, qb, e)])
            pp = jnp.exp2(s).astype(BF)
            if PST:
                slot = cnt[0] % (LAG + 1)
                cnt[0] += 1
                for t in range(TQ // 128):
                    p_s[slot * (TQ // 128) + t] = pp[:, t * 128:(t + 1) * 128]
                P[(us, qb, e, jb)] = slot
            else:
                P[(us, qb, e, jb)] = pp

        def do_pv(us, qb, e, jb):
            u = it * (HU // 2) + us
            h = 2 * u + e
            v = jnp.concatenate([vt_s[h * 16 + jb * (BJ // 128) + t] for t in range(BJ // 128)], axis=1)
            pp = P.pop((us, qb, e, jb))
            if PST:
                pp = jnp.concatenate([p_s[pp * (TQ // 128) + t] for t in range(TQ // 128)], axis=1)
            r = _dot(v, pp)
            key = (us, qb, e)
            acc[key] = acc[key] + r if key in acc else r
            if jb == S // BJ - 1 and e == 1:
                st[0] = jnp.maximum(st[0], store_pair(u, qb * TQ, TQ, acc.pop((us, qb, 0)), acc.pop((us, qb, 1))))

        for i, itx in enumerate(items):
            do_qk(*itx)
            if i - LAG >= 0:
                do_pv(*items[i - LAG])
        for i in range(len(items) - LAG, len(items)):
            do_pv(*items[i])
        return st[0]

    with scope('P2'):
        bad = lax.fori_loop(0, H // HU, attn_body, jnp.zeros((8, 128), F32)) if '2' in PH else jnp.zeros((8, 128), F32)
    flag = jnp.max(bad)

    @pl.when(flag > 0.0)
    def _slow():
        tq, bj = 256, 512
        def body(it, carry):
            u = it // (S // tq)
            q0 = pl.multiple_of((it % (S // tq)) * tq, tq)
            c = u // 3
            up = u % 3
            accs = []
            for e in range(2):
                p = 2 * up + e
                h = 2 * u + e
                qt = qtile(c, p, q0, tq, False)
                def mx(jb, m):
                    j0 = pl.multiple_of(jb * bj, bj)
                    s = _dot(k_s[c, pl.ds(j0, bj), :], qt)
                    return jnp.maximum(m, jnp.max(s, axis=0, keepdims=True))
                m = lax.fori_loop(0, S // bj, mx, jnp.full((1, tq), -jnp.inf, F32))
                def pv(jb, acc):
                    j0 = pl.multiple_of(jb * bj, bj)
                    s = _dot(k_s[c, pl.ds(j0, bj), :], qt)
                    pT = jnp.exp2(s - m).astype(BF)
                    v = jnp.concatenate([vt_s[h * 16 + jb * (bj // 128) + t] for t in range(bj // 128)], axis=1)
                    return acc + _dot(v, pT)
                accs.append(lax.fori_loop(0, S // bj, pv, jnp.zeros((24, tq), F32)))
            store_pair(u, q0, tq, accs[0], accs[1])
            return carry
        lax.fori_loop(0, (H // 2) * (S // tq), body, 0)

    wo_cp.wait()
    for cp in w13_cps:
        cp.wait()
    w2_cp.wait()
    lane_m = lax.broadcasted_iota(jnp.int32, (TM, 128), 1)

    hres = [None] * NOB
    hn = [None] * NOB
    act = [None] * NOB

    def outproj(rb):
        r0 = rb * TM
        oT = ot_s[:, r0:r0 + TM].astype(BF)
        a = lax.dot_general(oT, wo_s[...], (((0,), (0,)), ((), ())), preferred_element_type=F32)
        hres[rb] = x_s[r0:r0 + TM, :].astype(F32) + a

    def ln2(rb):
        hn[rb] = _ln(hres[rb]).astype(BF)

    def ffn_up(rb):
        gu = _dot_nt(hn[rb], w13_s[...])
        g = gu[:, 0:FM]
        up_ = gu[:, FM:2 * FM]
        act_main = (g * jax.nn.sigmoid(g) * up_).astype(BF)
        t = gu[:, 2 * FM:2 * FM + 128]
        act_last = jnp.where(lane_m < 64, t * jax.nn.sigmoid(t) * pltpu.roll(t, 64, 1), 0.0).astype(BF)
        act[rb] = jnp.concatenate([act_main, act_last], axis=1)

    def ffn_down(rb):
        y = hres[rb] + _dot(act[rb], w2_s[...])
        ob_s[rb] = y.astype(BF)
        out_cp[rb].start()

    with scope('P3'):
      if '3' not in PH:
        for rb in range(NOB):
            ob_s[rb] = xn_s[rb * TM:(rb + 1) * TM, :]
            out_cp[rb].start()
      else:
        outproj(0)
        if NOB > 1:
            outproj(1)
        ln2(0)
        for rb in range(NOB):
            ffn_up(rb)
            if rb + 1 < NOB:
                ln2(rb + 1)
            if rb + 2 < NOB:
                outproj(rb + 2)
            ffn_down(rb)
    for cp in out_cp:
        cp.wait()


@jax.jit
def pallas_sequential_preLN__softmax_full_mha__glu_gated_swiglu__prompt_kernel(A_x, A_wqkv, A_wo, B_x, B_w1, B_w3, B_w2):
    del B_x
    x = A_x.reshape(S, D)
    nsem = 8 + 9 + S // TM
    hbm = pl.BlockSpec(memory_space=pltpu.HBM)
    out = pl.pallas_call(
        _kernel,
        out_shape=jax.ShapeDtypeStruct((S, D), A_x.dtype),
        in_specs=[hbm] * 6,
        out_specs=hbm,
        scratch_shapes=[
            pltpu.VMEM((S, D), BF),
            pltpu.VMEM((S, D), BF),
            pltpu.VMEM((D, 3 * D), BF),
            pltpu.VMEM((D, D), BF),
            pltpu.VMEM((2 * F, D), BF),
            pltpu.VMEM((FP, D), BF),
            pltpu.VMEM((D, NSL * 128), BF),
            pltpu.VMEM((2 * D, D), BF),
            pltpu.VMEM((NSL, S, 128), BF),
            pltpu.VMEM((NSL, 128, S), F32),
            pltpu.VMEM((48, S), F32),
            pltpu.VMEM((H * 16, 24, 128), F32),
            pltpu.VMEM((D, S), F32),
            pltpu.VMEM((S // TM, TM, D), BF),
            pltpu.VMEM(((LAG + 1) * (TQ // 128), BJ, 128), BF),
            pltpu.SemaphoreType.DMA((nsem,)),
        ],
        compiler_params=pltpu.CompilerParams(vmem_limit_bytes=110 * 1024 * 1024),
        name="fused_block",
    )(x, A_wqkv, A_wo, B_w1.T, B_w3.T, B_w2)
    return out.reshape(A_x.shape)
```

```python
import functools

import jax
import jax.numpy as jnp
import numpy as np
from jax import lax
import jax.experimental.pallas as pl
import jax.experimental.pallas.tpu as pltpu

S, D, H, DH, F = 2048, 640, 32, 20, 1728
NSL = 6
FP = 1792
FM = 1664
EPS = 1e-5
QSCALE = float(DH ** -0.5 * np.log2(np.e))
B_MARGIN = 1.0 + 2.0 ** -6
L_LO, L_HI = 2.0 ** -90, 2.0 ** 60

TB = 512
RC, LC, AH = 128, 64, 2
TRS = 12
XP = (0, 512, 1024, 2048)
TQ, BJ = 512, 128
LAG, HU = 4, 4
TM, CR, DR = 512, 256, 128

BF = jnp.bfloat16
F32 = jnp.float32


def _ln(x):
    mu = jnp.mean(x, axis=-1, keepdims=True)
    xc = x - mu
    var = jnp.mean(xc * xc, axis=-1, keepdims=True)
    return xc * lax.rsqrt(var + EPS)


def _dot(a, b):
    return lax.dot_general(a, b, (((1,), (0,)), ((), ())), preferred_element_type=F32)


def _dot_nt(a, b):
    return lax.dot_general(a, b, (((1,), (1,)), ((), ())), preferred_element_type=F32)


def _dot_tn(a, b):
    return lax.dot_general(a, b, (((0,), (0,)), ((), ())), preferred_element_type=F32)


def _iota(shape, axis):
    return lax.broadcasted_iota(jnp.int32, shape, axis)


def _block_kernel(x_hbm, wqkv_hbm, wo_hbm, w1t_hbm, w3t_hbm, w2_hbm, out_hbm,
                  x_s, xn_s, wqkv_s, wo_s, w13_s, w2_s, wqvT_s,
                  k_s, q_s, nq_s, vt_s, ot_s, p_s, ob_s, sems):
    sem = iter(range(sems.shape[0]))

    def copy(src, dst):
        return pltpu.make_async_copy(src, dst, sems.at[next(sem)])

    def wcols(c0):
        return copy(wqkv_hbm.at[:, pl.ds(c0, D)], wqkv_s.at[:, pl.ds(c0, D)])

    x_cp = [copy(x_hbm.at[pl.ds(a, b - a)], x_s.at[pl.ds(a, b - a)])
            for a, b in zip(XP[:-1], XP[1:])]
    wq_cp, wk_cp, wv_cp = wcols(0), wcols(D), wcols(2 * D)
    ffn_cps = [
        copy(wo_hbm, wo_s),
        copy(w1t_hbm.at[pl.ds(0, FM)], w13_s.at[pl.ds(0, FM)]),
        copy(w3t_hbm.at[pl.ds(0, FM)], w13_s.at[pl.ds(FM, FM)]),
        copy(w1t_hbm.at[pl.ds(FM, F - FM)], w13_s.at[pl.ds(2 * FM, F - FM)]),
        copy(w3t_hbm.at[pl.ds(FM, F - FM)], w13_s.at[pl.ds(FM + F, F - FM)]),
        copy(w2_hbm, w2_s.at[pl.ds(0, F)]),
    ]
    NOB = S // TM
    out_cp = [copy(ob_s.at[b], out_hbm.at[pl.ds(b * TM, TM)]) for b in range(NOB - 1)]
    last_cp = [copy(ob_s.at[NOB - 1, pl.ds(k * DR, DR)],
                    out_hbm.at[pl.ds((NOB - 1) * TM + k * DR, DR)]) for k in range(TM // DR)]

    x_cp[0].start()
    wk_cp.start()
    for cp in x_cp[1:]:
        cp.start()
    wq_cp.start()
    wv_cp.start()
    for cp in ffn_cps:
        cp.start(priority=1)
    w2_s[F:FP, :] = jnp.zeros((FP - F, D), BF)

    rk, lk = _iota((48, NSL * 128), 0), _iota((48, NSL * 128), 1)
    segk = jnp.where((lk // 128 == rk // 8) & ((lk % 128) // DH == rk % 8) & (lk % 128 < 120),
                     1.0, 0.0).astype(BF)
    rq, fq = _iota((48, D), 0), _iota((48, D), 1)
    segq = jnp.where(((rq % 8) < 6) & (fq // DH == 6 * (rq // 8) + (rq % 8)), 1.0, 0.0).astype(BF)
    lane_k = _iota((RC, 128), 1)
    sub8 = _iota((8, TB), 0)

    def ln_chunk(i):
        for t0 in range(i * RC, (i + 1) * RC, LC):
            xn_s[t0:t0 + LC, :] = _ln(x_s[t0:t0 + LC, :].astype(F32)).astype(BF)

    def k_chunk(i):
        t0 = i * RC
        kk = _dot(xn_s[t0:t0 + RC, :], wqkv_s[:, D:2 * D]).astype(BF)
        kk = jnp.concatenate([kk, jnp.zeros((RC, 128), BF)], axis=1)
        for c in range(NSL):
            kc = kk[:, 120 * c:120 * c + 128]
            k_s[c, t0:t0 + RC, :] = jnp.where(lane_k >= 120, jnp.ones_like(kc), kc)

    def w_transpose(j):
        c0 = j * 128 if j < 5 else 2 * D + (j - 5) * 128
        wqvT_s[j * 128:(j + 1) * 128, :] = wqkv_s[:, c0:c0 + 128].T

    def qv_block(b):
        t0 = b * TB
        qv = _dot_nt(wqvT_s[...], xn_s[t0:t0 + TB, :])
        qf = (qv[0:D, :] * QSCALE).astype(BF).astype(F32)
        nq_s[:, t0:t0 + TB] = _dot(segq, (qf * qf).astype(BF))
        for c in range(NSL):
            lo, hi = 120 * c, min(120 * c + 120, D)
            q_s[c, 0:hi - lo, t0:t0 + TB] = qf[lo:hi, :]
            if hi - lo < 120:
                q_s[c, hi - lo:120, t0:t0 + TB] = jnp.zeros((120 - (hi - lo), TB), F32)
        vT = qv[D:2 * D, :].astype(BF).astype(F32)
        for h in range(H):
            a = 8 * ((DH * h) // 8)
            if h % 2 == 0:
                blk = jnp.concatenate(
                    [vT[a:a + 16, :], jnp.where(sub8 < 4, vT[a + 16:a + 24, :], 1.0)], axis=0)
            else:
                blk = jnp.concatenate(
                    [jnp.where(sub8 < 4, 1.0, vT[a:a + 8, :]), vT[a + 8:a + 24, :]], axis=0)
            for jt in range(TB // 128):
                vt_s[h * 16 + b * (TB // 128) + jt] = blk[:, jt * 128:(jt + 1) * 128]

    def k_norms(b, kmx):
        t0 = b * TB
        kf = jnp.concatenate([k_s[c, t0:t0 + TB, :] for c in range(NSL)], axis=1).astype(F32)
        nsq = _dot_nt(segk, (kf * kf).astype(BF))
        m = nsq[:, 0:128]
        for t in range(1, TB // 128):
            m = jnp.maximum(m, nsq[:, t * 128:(t + 1) * 128])
        return jnp.maximum(kmx, m)

    arrived = [0]

    def need_x(i):
        while XP[arrived[0]] < (i + 1) * RC:
            x_cp[arrived[0]].wait()
            arrived[0] += 1

    NC = S // RC
    for i in range(AH):
        need_x(i)
        ln_chunk(i)
    wk_cp.wait()
    pending = list(range(2 * D // 128))
    for i in range(NC):
        if i + AH < NC:
            need_x(i + AH)
        if i == TRS:
            wq_cp.wait()
            wv_cp.wait()
        k_chunk(i)
        if i + AH < NC:
            ln_chunk(i + AH)
        if i >= TRS:
            n = -(-len(pending) // (NC - i))
            for j in pending[:n]:
                w_transpose(j)
            pending = pending[n:]
    kmx = jnp.zeros((48, 128), F32)
    for b in range(S // TB):
        qv_block(b)
        kmx = k_norms(b, kmx)
    for c in range(NSL):
        kmax = jnp.sqrt(jnp.max(kmx[8 * c:8 * c + 8, :], axis=1, keepdims=True))
        q_s[c, 120:128, :] = -(jnp.sqrt(nq_s[8 * c:8 * c + 8, :]) * kmax) * B_MARGIN

    qrow = _iota((128, 128), 0)

    def q_tile(c, p, q0, tq, with_bound):
        m = (qrow >= DH * p) & (qrow < DH * p + DH)
        if with_bound:
            m = m | (qrow == 120 + p)
        parts = [jnp.where(m, q_s[c, :, pl.ds(q0 + t * 128, 128)], 0.0).astype(BF)
                 for t in range(tq // 128)]
        return jnp.concatenate(parts, axis=1)

    def store_pair(u, q0, tq, acc_e, acc_o):
        sub = _iota((8, tq), 0)
        le = jnp.broadcast_to(acc_e[20:21, :], (8, tq))
        lo = jnp.broadcast_to(acc_o[0:1, :], (8, tq))
        ie, io = 1.0 / le, 1.0 / lo
        mid = jnp.where(sub < 4, acc_e[16:24, :] * ie, acc_o[0:8, :] * io)
        blk = jnp.concatenate([acc_e[0:8, :] * ie, acc_e[8:16, :] * ie, mid,
                               acc_o[8:16, :] * io, acc_o[16:24, :] * io], axis=0)
        ot_s[pl.ds(pl.multiple_of(u * 40, 8), 40), pl.ds(q0, tq)] = blk
        ok = (le >= L_LO) & (le <= L_HI) & (lo >= L_LO) & (lo <= L_HI)
        unsafe = jnp.where(ok, 0.0, 1.0)
        r = unsafe[:, 0:128]
        for t in range(1, tq // 128):
            r = jnp.maximum(r, unsafe[:, t * 128:(t + 1) * 128])
        return r

    def attn_trip(it, unsafe):
        NT = TQ // 128
        steps = [(us, qb, e, jb) for us in range(HU // 2) for qb in range(S // TQ)
                 for e in range(2) for jb in range(S // BJ)]
        qts, slot_of, acc = {}, {}, {}
        flags = [unsafe]

        def qk(n, us, qb, e, jb):
            u = it * (HU // 2) + us
            c, p = u // 3, 2 * (u % 3) + e
            if (us, qb, e) not in qts:
                qts[us, qb, e] = q_tile(c, p, qb * TQ, TQ, True)
            s = _dot(k_s[c, jb * BJ:(jb + 1) * BJ, :], qts[us, qb, e])
            pT = jnp.exp2(s).astype(BF)
            slot = slot_of[us, qb, e, jb] = n % (LAG + 1)
            for t in range(NT):
                p_s[slot * NT + t] = pT[:, t * 128:(t + 1) * 128]

        def pv(us, qb, e, jb):
            u = it * (HU // 2) + us
            slot = slot_of.pop((us, qb, e, jb))
            pT = jnp.concatenate([p_s[slot * NT + t] for t in range(NT)], axis=1)
            r = _dot(vt_s[(2 * u + e) * 16 + jb], pT)
            acc[us, qb, e] = acc[us, qb, e] + r if jb else r
            if jb == S // BJ - 1 and e == 1:
                flags.append(jnp.maximum(flags.pop(), store_pair(
                    u, qb * TQ, TQ, acc.pop((us, qb, 0)), acc.pop((us, qb, 1)))))

        for n, step in enumerate(steps):
            qk(n, *step)
            if n >= LAG:
                pv(*steps[n - LAG])
        for step in steps[len(steps) - LAG:]:
            pv(*step)
        return flags[0]

    unsafe = lax.fori_loop(0, H // HU, attn_trip, jnp.zeros((8, 128), F32))

    @pl.when(jnp.max(unsafe) > 0.0)
    def _exact_max_fallback():
        tq, bj = 256, 512

        def pair(it, carry):
            u = it // (S // tq)
            q0 = pl.multiple_of((it % (S // tq)) * tq, tq)
            c = u // 3
            accs = []
            for e in range(2):
                h = 2 * u + e
                qt = q_tile(c, 2 * (u % 3) + e, q0, tq, False)

                def row_max(jb, m):
                    s = _dot(k_s[c, pl.ds(pl.multiple_of(jb * bj, bj), bj), :], qt)
                    return jnp.maximum(m, jnp.max(s, axis=0, keepdims=True))

                m = lax.fori_loop(0, S // bj, row_max, jnp.full((1, tq), -jnp.inf, F32))

                def accumulate(jb, o):
                    s = _dot(k_s[c, pl.ds(pl.multiple_of(jb * bj, bj), bj), :], qt)
                    pT = jnp.exp2(s - m).astype(BF)
                    v = jnp.concatenate([vt_s[h * 16 + jb * (bj // 128) + t]
                                         for t in range(bj // 128)], axis=1)
                    return o + _dot(v, pT)

                accs.append(lax.fori_loop(0, S // bj, accumulate, jnp.zeros((24, tq), F32)))
            store_pair(u, q0, tq, accs[0], accs[1])
            return carry

        lax.fori_loop(0, (H // 2) * (S // tq), pair, 0)

    for cp in ffn_cps:
        cp.wait()
    lane_m = _iota((TM, 128), 1)
    hres, hn, act = {}, {}, {}
    CPB = TM // CR

    def out_proj(i):
        r0 = i * CR
        a = _dot_tn(ot_s[:, r0:r0 + CR].astype(BF), wo_s[...])
        hres[i] = x_s[r0:r0 + CR, :].astype(F32) + a

    def ln2(i):
        hn[i] = _ln(hres[i]).astype(BF)

    def ffn_up(b):
        h = jnp.concatenate([hn.pop(b * CPB + k) for k in range(CPB)], axis=0)
        gu = _dot_nt(h, w13_s[...])
        g, up = gu[:, 0:FM], gu[:, FM:2 * FM]
        main = (g * jax.nn.sigmoid(g) * up).astype(BF)
        t = gu[:, 2 * FM:2 * FM + 128]
        tail = jnp.where(lane_m < 64, t * jax.nn.sigmoid(t) * pltpu.roll(t, 64, 1), 0.0)
        act[b] = jnp.concatenate([main, tail.astype(BF)], axis=1)

    def ffn_down(b):
        a = act.pop(b)
        h = jnp.concatenate([hres.pop(b * CPB + k) for k in range(CPB)], axis=0)
        if b < NOB - 1:
            ob_s[b] = (h + _dot(a, w2_s[...])).astype(BF)
            out_cp[b].start()
        else:
            for k in range(TM // DR):
                rows = slice(k * DR, (k + 1) * DR)
                ob_s[b, rows, :] = (h[rows] + _dot(a[rows], w2_s[...])).astype(BF)
                last_cp[k].start()

    for i in range(CPB + 1):
        out_proj(i)
        if i >= 1:
            ln2(i - 1)
    nxt = CPB + 1
    for b in range(NOB):
        ffn_up(b)
        if b + 1 < NOB:
            for i in range((b + 1) * CPB, (b + 2) * CPB):
                if nxt < S // CR and nxt <= i + 1:
                    out_proj(nxt)
                    nxt += 1
                ln2(i)
        ffn_down(b)
    for cp in out_cp + last_cp:
        cp.wait()


@jax.jit
def pallas_sequential_preLN__softmax_full_mha__glu_gated_swiglu__prompt_kernel(A_x, A_wqkv, A_wo, B_x, B_w1, B_w3, B_w2):
    del B_x
    hbm = pl.BlockSpec(memory_space=pltpu.HBM)
    n_sems = (len(XP) - 1) + 3 + 6 + (S // TM - 1) + TM // DR
    out = pl.pallas_call(
        _block_kernel,
        out_shape=jax.ShapeDtypeStruct((S, D), A_x.dtype),
        in_specs=[hbm] * 6,
        out_specs=hbm,
        scratch_shapes=[
            pltpu.VMEM((S, D), BF),
            pltpu.VMEM((S, D), BF),
            pltpu.VMEM((D, 3 * D), BF),
            pltpu.VMEM((D, D), BF),
            pltpu.VMEM((2 * F, D), BF),
            pltpu.VMEM((FP, D), BF),
            pltpu.VMEM((2 * D, D), BF),
            pltpu.VMEM((NSL, S, 128), BF),
            pltpu.VMEM((NSL, 128, S), F32),
            pltpu.VMEM((48, S), F32),
            pltpu.VMEM((H * 16, 24, 128), F32),
            pltpu.VMEM((D, S), F32),
            pltpu.VMEM(((LAG + 1) * (TQ // 128), BJ, 128), BF),
            pltpu.VMEM((S // TM, TM, D), BF),
            pltpu.SemaphoreType.DMA((n_sems,)),
        ],
        compiler_params=pltpu.CompilerParams(vmem_limit_bytes=110 * 1024 * 1024),
        name="fused_block",
    )(A_x.reshape(S, D), A_wqkv, A_wo, B_w1.T, B_w3.T, B_w2)
    return out.reshape(A_x.shape)
```

```python
import jax
import jax.numpy as jnp
import numpy as np
from jax import lax
import jax.experimental.pallas as pl
import jax.experimental.pallas.tpu as pltpu

S, D, H, DH, F = 2048, 640, 32, 20, 1728
NSL = 6
FP = 1792
FM = 1664
EPS = 1e-5
QSCALE = float(DH ** -0.5 * np.log2(np.e))
B_MARGIN = 1.0 + 2.0 ** -6
L_LO, L_HI = 2.0 ** -90, 2.0 ** 60

TB = 512
RC, LC, AH = 64, 32, 4
TRS = 24
XP = (0, 512, 1024, 2048)
TQ, BJ = 512, 128
LAG, HU = 8, 4
TM, CR, DR = 1024, 256, 64

BF = jnp.bfloat16
F32 = jnp.float32


def _ln(x):
    mu = jnp.mean(x, axis=-1, keepdims=True)
    xc = x - mu
    var = jnp.mean(xc * xc, axis=-1, keepdims=True)
    return xc * lax.rsqrt(var + EPS)


def _dot(a, b):
    return lax.dot_general(a, b, (((1,), (0,)), ((), ())), preferred_element_type=F32)


def _dot_nt(a, b):
    return lax.dot_general(a, b, (((1,), (1,)), ((), ())), preferred_element_type=F32)


def _dot_tn(a, b):
    return lax.dot_general(a, b, (((0,), (0,)), ((), ())), preferred_element_type=F32)


def _iota(shape, axis):
    return lax.broadcasted_iota(jnp.int32, shape, axis)


def _block_kernel(x_hbm, wqkv_hbm, wo_hbm, w1t_hbm, w3t_hbm, w2_hbm, out_hbm,
                  x_s, xn_s, wqkv_s, wo_s, w13_s, w2_s, wqvT_s,
                  k_s, q_s, nq_s, vt_s, ot_s, p_s, ob_s, sems):
    sem = iter(range(sems.shape[0]))

    def copy(src, dst):
        return pltpu.make_async_copy(src, dst, sems.at[next(sem)])

    def wcols(c0):
        return copy(wqkv_hbm.at[:, pl.ds(c0, D)], wqkv_s.at[:, pl.ds(c0, D)])

    x_cp = [copy(x_hbm.at[pl.ds(a, b - a)], x_s.at[pl.ds(a, b - a)])
            for a, b in zip(XP[:-1], XP[1:])]
    wq_cp, wk_cp, wv_cp = wcols(0), wcols(D), wcols(2 * D)
    ffn_cps = [
        copy(wo_hbm, wo_s),
        copy(w1t_hbm.at[pl.ds(0, FM)], w13_s.at[pl.ds(0, FM)]),
        copy(w3t_hbm.at[pl.ds(0, FM)], w13_s.at[pl.ds(FM, FM)]),
        copy(w1t_hbm.at[pl.ds(FM, F - FM)], w13_s.at[pl.ds(2 * FM, F - FM)]),
        copy(w3t_hbm.at[pl.ds(FM, F - FM)], w13_s.at[pl.ds(FM + F, F - FM)]),
        copy(w2_hbm, w2_s.at[pl.ds(0, F)]),
    ]
    NOB = S // TM
    out_cp = [copy(ob_s.at[b], out_hbm.at[pl.ds(b * TM, TM)]) for b in range(NOB - 1)]
    last_cp = [copy(ob_s.at[NOB - 1, pl.ds(k * DR, DR)],
                    out_hbm.at[pl.ds((NOB - 1) * TM + k * DR, DR)]) for k in range(TM // DR)]

    x_cp[0].start()
    wk_cp.start()
    for cp in x_cp[1:]:
        cp.start()
    wq_cp.start()
    wv_cp.start()
    w2_s[F:FP, :] = jnp.zeros((FP - F, D), BF)
    for cp in ffn_cps:
        cp.start(priority=1)

    rk, lk = _iota((48, NSL * 128), 0), _iota((48, NSL * 128), 1)
    segk = jnp.where((lk // 128 == rk // 8) & ((lk % 128) // DH == rk % 8) & (lk % 128 < 120),
                     1.0, 0.0).astype(BF)
    rq, fq = _iota((48, D), 0), _iota((48, D), 1)
    segq = jnp.where(((rq % 8) < 6) & (fq // DH == 6 * (rq // 8) + (rq % 8)), 1.0, 0.0).astype(BF)
    lane_k = _iota((RC, 128), 1)
    sub8 = _iota((8, TB), 0)

    def ln_chunk(i):
        for t0 in range(i * RC, (i + 1) * RC, LC):
            xn_s[t0:t0 + LC, :] = _ln(x_s[t0:t0 + LC, :].astype(F32)).astype(BF)

    def k_matmul(i):
        return _dot(xn_s[i * RC:(i + 1) * RC, :], wqkv_s[:, D:2 * D])

    def k_store(i, kk):
        t0 = i * RC
        kk = jnp.concatenate([kk.astype(BF), jnp.zeros((RC, 128), BF)], axis=1)
        for c in range(NSL):
            kc = kk[:, 120 * c:120 * c + 128]
            k_s[c, t0:t0 + RC, :] = jnp.where(lane_k >= 120, jnp.ones_like(kc), kc)

    def w_transpose(j):
        c0 = j * 128 if j < 5 else 2 * D + (j - 5) * 128
        wqvT_s[j * 128:(j + 1) * 128, :] = wqkv_s[:, c0:c0 + 128].T

    def qv_block(b):
        t0 = b * TB
        qv = _dot_nt(wqvT_s[...], xn_s[t0:t0 + TB, :])
        qf = (qv[0:D, :] * QSCALE).astype(BF).astype(F32)
        nq_s[:, t0:t0 + TB] = _dot(segq, (qf * qf).astype(BF))
        for c in range(NSL):
            lo, hi = 120 * c, min(120 * c + 120, D)
            q_s[c, 0:hi - lo, t0:t0 + TB] = qf[lo:hi, :]
            if hi - lo < 120:
                q_s[c, hi - lo:120, t0:t0 + TB] = jnp.zeros((120 - (hi - lo), TB), F32)
        vT = qv[D:2 * D, :].astype(BF).astype(F32)
        for h in range(H):
            a = 8 * ((DH * h) // 8)
            if h % 2 == 0:
                blk = jnp.concatenate(
                    [vT[a:a + 16, :], jnp.where(sub8 < 4, vT[a + 16:a + 24, :], 1.0)], axis=0)
            else:
                blk = jnp.concatenate(
                    [jnp.where(sub8 < 4, 1.0, vT[a:a + 8, :]), vT[a + 8:a + 24, :]], axis=0)
            for jt in range(TB // 128):
                vt_s[h * 16 + b * (TB // 128) + jt] = blk[:, jt * 128:(jt + 1) * 128]

    def k_norms(b, kmx):
        t0 = b * TB
        kf = jnp.concatenate([k_s[c, t0:t0 + TB, :] for c in range(NSL)], axis=1).astype(F32)
        nsq = _dot_nt(segk, (kf * kf).astype(BF))
        m = nsq[:, 0:128]
        for t in range(1, TB // 128):
            m = jnp.maximum(m, nsq[:, t * 128:(t + 1) * 128])
        return jnp.maximum(kmx, m)

    arrived = [0]

    def need_x(i):
        while XP[arrived[0]] < (i + 1) * RC:
            x_cp[arrived[0]].wait()
            arrived[0] += 1

    NC = S // RC
    for i in range(AH):
        need_x(i)
        ln_chunk(i)
    wk_cp.wait()
    pending = list(range(2 * D // 128))
    k_prev = None
    for i in range(NC):
        if i + AH < NC:
            need_x(i + AH)
        if i == TRS:
            wq_cp.wait()
            wv_cp.wait()
        k_cur = k_matmul(i)
        if i:
            k_store(i - 1, k_prev)
        k_prev = k_cur
        if i + AH < NC:
            ln_chunk(i + AH)
        if i >= TRS:
            n = -(-len(pending) // (NC - i))
            for j in pending[:n]:
                w_transpose(j)
            pending = pending[n:]
    k_store(NC - 1, k_prev)
    kmx = jnp.zeros((48, 128), F32)
    for b in range(S // TB):
        qv_block(b)
        kmx = k_norms(b, kmx)
    for c in range(NSL):
        kmax = jnp.sqrt(jnp.max(kmx[8 * c:8 * c + 8, :], axis=1, keepdims=True))
        q_s[c, 120:128, :] = -(jnp.sqrt(nq_s[8 * c:8 * c + 8, :]) * kmax) * B_MARGIN

    qrow = _iota((128, 128), 0)

    def q_tile(c, p, q0, tq, with_bound):
        m = (qrow >= DH * p) & (qrow < DH * p + DH)
        if with_bound:
            m = m | (qrow == 120 + p)
        parts = [jnp.where(m, q_s[c, :, pl.ds(q0 + t * 128, 128)], 0.0).astype(BF)
                 for t in range(tq // 128)]
        return jnp.concatenate(parts, axis=1)

    def store_pair(u, q0, tq, acc_e, acc_o):
        sub = _iota((8, tq), 0)
        le = jnp.broadcast_to(acc_e[20:21, :], (8, tq))
        lo = jnp.broadcast_to(acc_o[0:1, :], (8, tq))
        ie, io = 1.0 / le, 1.0 / lo
        mid = jnp.where(sub < 4, acc_e[16:24, :] * ie, acc_o[0:8, :] * io)
        blk = jnp.concatenate([acc_e[0:8, :] * ie, acc_e[8:16, :] * ie, mid,
                               acc_o[8:16, :] * io, acc_o[16:24, :] * io], axis=0)
        ot_s[pl.ds(pl.multiple_of(u * 40, 8), 40), pl.ds(q0, tq)] = blk
        ok = (le >= L_LO) & (le <= L_HI) & (lo >= L_LO) & (lo <= L_HI)
        unsafe = jnp.where(ok, 0.0, 1.0)
        r = unsafe[:, 0:128]
        for t in range(1, tq // 128):
            r = jnp.maximum(r, unsafe[:, t * 128:(t + 1) * 128])
        return r

    def attn_trip(it, unsafe):
        NT = TQ // 128
        steps = [(us, qb, e, jb) for us in range(HU // 2) for qb in range(S // TQ)
                 for e in range(2) for jb in range(S // BJ)]
        qts, slot_of, acc = {}, {}, {}
        flags = [unsafe]

        def qk(n, us, qb, e, jb):
            u = it * (HU // 2) + us
            c, p = u // 3, 2 * (u % 3) + e
            if (us, qb, e) not in qts:
                qts[us, qb, e] = q_tile(c, p, qb * TQ, TQ, True)
            s = _dot(k_s[c, jb * BJ:(jb + 1) * BJ, :], qts[us, qb, e])
            pT = jnp.exp2(s).astype(BF)
            slot = slot_of[us, qb, e, jb] = n % (LAG + 1)
            for t in range(NT):
                p_s[slot * NT + t] = pT[:, t * 128:(t + 1) * 128]

        def pv(us, qb, e, jb):
            u = it * (HU // 2) + us
            slot = slot_of.pop((us, qb, e, jb))
            pT = jnp.concatenate([p_s[slot * NT + t] for t in range(NT)], axis=1)
            r = _dot(vt_s[(2 * u + e) * 16 + jb], pT)
            acc[us, qb, e] = acc[us, qb, e] + r if jb else r
            if jb == S // BJ - 1 and e == 1:
                flags.append(jnp.maximum(flags.pop(), store_pair(
                    u, qb * TQ, TQ, acc.pop((us, qb, 0)), acc.pop((us, qb, 1)))))

        for n, step in enumerate(steps):
            qk(n, *step)
            if n >= LAG:
                pv(*steps[n - LAG])
        for step in steps[len(steps) - LAG:]:
            pv(*step)
        return flags[0]

    unsafe = lax.fori_loop(0, H // HU, attn_trip, jnp.zeros((8, 128), F32))

    @pl.when(jnp.max(unsafe) > 0.0)
    def _exact_max_fallback():
        tq, bj = 256, 512

        def pair(it, carry):
            u = it // (S // tq)
            q0 = pl.multiple_of((it % (S // tq)) * tq, tq)
            c = u // 3
            accs = []
            for e in range(2):
                h = 2 * u + e
                qt = q_tile(c, 2 * (u % 3) + e, q0, tq, False)

                def row_max(jb, m):
                    s = _dot(k_s[c, pl.ds(pl.multiple_of(jb * bj, bj), bj), :], qt)
                    return jnp.maximum(m, jnp.max(s, axis=0, keepdims=True))

                m = lax.fori_loop(0, S // bj, row_max, jnp.full((1, tq), -jnp.inf, F32))

                def accumulate(jb, o):
                    s = _dot(k_s[c, pl.ds(pl.multiple_of(jb * bj, bj), bj), :], qt)
                    pT = jnp.exp2(s - m).astype(BF)
                    v = jnp.concatenate([vt_s[h * 16 + jb * (bj // 128) + t]
                                         for t in range(bj // 128)], axis=1)
                    return o + _dot(v, pT)

                accs.append(lax.fori_loop(0, S // bj, accumulate, jnp.zeros((24, tq), F32)))
            store_pair(u, q0, tq, accs[0], accs[1])
            return carry

        lax.fori_loop(0, (H // 2) * (S // tq), pair, 0)

    for cp in ffn_cps:
        cp.wait()
    lane_m = _iota((TM, 128), 1)
    hres, hn, act = {}, {}, {}
    CPB = TM // CR

    def out_proj(i):
        r0 = i * CR
        a = _dot_tn(ot_s[:, r0:r0 + CR].astype(BF), wo_s[...])
        hres[i] = x_s[r0:r0 + CR, :].astype(F32) + a

    def ln2(i):
        hn[i] = _ln(hres[i]).astype(BF)

    def ffn_up(b):
        h = jnp.concatenate([hn.pop(b * CPB + k) for k in range(CPB)], axis=0)
        gu = _dot_nt(h, w13_s[...])
        g, up = gu[:, 0:FM], gu[:, FM:2 * FM]
        main = (g * jax.nn.sigmoid(g) * up).astype(BF)
        t = gu[:, 2 * FM:2 * FM + 128]
        tail = jnp.where(lane_m < 64, t * jax.nn.sigmoid(t) * pltpu.roll(t, 64, 1), 0.0)
        act[b] = jnp.concatenate([main, tail.astype(BF)], axis=1)

    def ffn_down(b):
        a = act.pop(b)
        h = jnp.concatenate([hres.pop(b * CPB + k) for k in range(CPB)], axis=0)
        if b < NOB - 1:
            ob_s[b] = (h + _dot(a, w2_s[...])).astype(BF)
            out_cp[b].start()
        else:
            for k in range(TM // DR):
                rows = slice(k * DR, (k + 1) * DR)
                ob_s[b, rows, :] = (h[rows] + _dot(a[rows], w2_s[...])).astype(BF)
                last_cp[k].start()

    for i in range(CPB + 1):
        out_proj(i)
        if i >= 1:
            ln2(i - 1)
    nxt = CPB + 1
    for b in range(NOB):
        ffn_up(b)
        if b + 1 < NOB:
            for i in range((b + 1) * CPB, (b + 2) * CPB):
                if nxt < S // CR and nxt <= i + 1:
                    out_proj(nxt)
                    nxt += 1
                ln2(i)
        ffn_down(b)
    for cp in out_cp + last_cp:
        cp.wait()


@jax.jit
def pallas_sequential_preLN__softmax_full_mha__glu_gated_swiglu__prompt_kernel(A_x, A_wqkv, A_wo, B_x, B_w1, B_w3, B_w2):
    del B_x
    hbm = pl.BlockSpec(memory_space=pltpu.HBM)
    n_sems = (len(XP) - 1) + 3 + 6 + (S // TM - 1) + TM // DR
    out = pl.pallas_call(
        _block_kernel,
        out_shape=jax.ShapeDtypeStruct((S, D), A_x.dtype),
        in_specs=[hbm] * 6,
        out_specs=hbm,
        scratch_shapes=[
            pltpu.VMEM((S, D), BF),
            pltpu.VMEM((S, D), BF),
            pltpu.VMEM((D, 3 * D), BF),
            pltpu.VMEM((D, D), BF),
            pltpu.VMEM((2 * F, D), BF),
            pltpu.VMEM((FP, D), BF),
            pltpu.VMEM((2 * D, D), BF),
            pltpu.VMEM((NSL, S, 128), BF),
            pltpu.VMEM((NSL, 128, S), F32),
            pltpu.VMEM((48, S), F32),
            pltpu.VMEM((H * 16, 24, 128), F32),
            pltpu.VMEM((D, S), F32),
            pltpu.VMEM(((LAG + 1) * (TQ // 128), BJ, 128), BF),
            pltpu.VMEM((S // TM, TM, D), BF),
            pltpu.SemaphoreType.DMA((n_sems,)),
        ],
        compiler_params=pltpu.CompilerParams(vmem_limit_bytes=110 * 1024 * 1024),
        name="fused_block",
    )(A_x.reshape(S, D), A_wqkv, A_wo, B_w1.T, B_w3.T, B_w2)
    return out.reshape(A_x.shape)
```
